```python
import os as _os
_os.environ.setdefault("JAX_PLATFORMS", "cpu")
import jax
import jax.numpy as jnp

def _softmax(x, axis=-1):
    return jax.nn.softmax(x, axis=axis)
def _gelu(x):
    return jax.nn.gelu(x, approximate=True)
def _silu(x):
    return jax.nn.silu(x)
def _sigmoid(x):
    return jax.nn.sigmoid(x)
def _layernorm(x, axis=-1, eps=1e-5):
    m = jnp.mean(x, axis=axis, keepdims=True)
    v = jnp.var(x, axis=axis, keepdims=True)
    return (x - m) / jnp.sqrt(v + eps)
def _scatter_add(tgt, idx, src, axis=0):
    return tgt.at[idx].add(src)
def _segment_sum(src, seg, n):
    return jax.ops.segment_sum(src, seg, n)
class _Rng:
    def __init__(self, key):
        self._k = key
    def _next(self):
        self._k, sub = jax.random.split(self._k)
        return sub
    def normal(self, shape):
        return jax.random.normal(self._next(), shape, dtype=jnp.bfloat16)
    def randint(self, lo, hi, shape):
        return jax.random.randint(self._next(), shape, lo, hi, dtype=jnp.int32)
    def uniform(self, shape, lo=0.0, hi=1.0):
        return jax.random.uniform(self._next(), shape, jnp.bfloat16, lo, hi)
    def permutation(self, n):
        return jax.random.permutation(self._next(), n)


kernel_name = 'parallel_sum__softmax_full_mha__swiglu_ffn__prompt'

def setup_inputs():
    _rng = _Rng(jax.random.key(int.from_bytes(__import__("os").urandom(4), "little")))
    _w = (lambda a: (lambda t: t.astype(jnp.bfloat16) if jnp.issubdtype(t.dtype, jnp.floating) else t)(jnp.asarray(a)))
    def _A_setup():
        B, S, D = 1, 2048, 640
        return {
            "x": _w((lambda *s: _rng.normal(s) * 0.05)(B, S, D)),
            "wqkv": _w((lambda *s: _rng.normal(s) * 0.1)(D, 3 * D)),
            "wo": _w((lambda *s: _rng.normal(s) * 0.05)(D, D)),
        }
    _A_in = _A_setup()

    def _B_setup():
        B, S, D, F = 1, 2048, 640, 1536
        return {
            "x": _w((lambda *s: _rng.normal(s) * 0.05)(B, S, D)),
            "w_gate": _w((lambda *s: _rng.normal(s) * 0.05)(D, F)),
            "w_up": _w((lambda *s: _rng.normal(s) * 0.05)(D, F)),
            "w_down": _w((lambda *s: _rng.normal(s) * 0.05)(F, D)),
        }
    _B_in = _B_setup()

    return {
        "A_x": _A_in["x"],
        "A_wqkv": _A_in["wqkv"],
        "A_wo": _A_in["wo"],
        "B_x": _B_in["x"],
        "B_w_gate": _B_in["w_gate"],
        "B_w_up": _B_in["w_up"],
        "B_w_down": _B_in["w_down"],
    }

def reference(A_x, A_wqkv, A_wo, B_x, B_w_gate, B_w_up, B_w_down):
    def _A_ref(x, wqkv, wo):
        B, S, D = x.shape
        H = 32; Dh = D // H
        qkv = (lambda x, *d: x.transpose(*d))((x @ wqkv).reshape(B, S, 3, H, Dh), 2, 0, 3, 1, 4)
        q, k, v = qkv[0], qkv[1], qkv[2]
        scale = Dh ** -0.5
        scores = jnp.einsum("bhqd,bhkd->bhqk", q, k) * scale
        p = _softmax(scores, axis=-1)
        o = jnp.einsum("bhqk,bhkd->bhqd", p, v)
        return (lambda x, *d: x.transpose(*d))(o, 0, 2, 1, 3).reshape(B, S, D) @ wo

    def _B_ref(x, w_gate, w_up, w_down):
        g = _silu(x @ w_gate)
        u = x @ w_up
        return (g * u) @ w_down

    x = A_x
    xn = _layernorm(x, axis=-1)
    return x + _A_ref(xn, A_wqkv, A_wo) + _B_ref(xn, B_w_gate, B_w_up, B_w_down)
```

```python
import math

import jax
import jax.numpy as jnp
from jax import lax
import jax.experimental.pallas as pl
import jax.experimental.pallas.tpu as pltpu

S, D, F = 2048, 640, 1536
H, DH = 32, 20
HPG = 6
NG = -(-H // HPG)
GW = HPG * DH
DPAD = 768
BQ = 1024
NQB = S // BQ
CK = 128
RA = 512
RC = 512
F32, BF16 = jnp.float32, jnp.bfloat16
Q_SCALE = DH ** -0.5 * math.log2(math.e)


def _dot(a, b):
    return jnp.dot(a, b, preferred_element_type=F32)


def _kernel(x_hbm, wqkv_hbm, wo_hbm, wg_hbm, wu_hbm, wd_hbm, out_hbm,
            x_v, wqkv_v, wo_v, wg_v, wu_v, wd_v, out_v,
            xn_v, wk_v, wqvt_v, k_v, qt_v, vt_v, va_v, ot_v, sa_v, sb_v, m_v,
            in_sem, out_sem):
    x_copies = [
        pltpu.make_async_copy(x_hbm.at[pl.ds(r * RA, RA)], x_v.at[pl.ds(r * RA, RA)], in_sem.at[r])
        for r in range(S // RA)
    ]
    w_copies = [
        pltpu.make_async_copy(src, dst, in_sem.at[S // RA + i])
        for i, (src, dst) in enumerate(
            [(wqkv_hbm, wqkv_v), (wo_hbm, wo_v), (wg_hbm, wg_v), (wu_hbm, wu_v), (wd_hbm, wd_v)])
    ]
    w_copies[0].start()
    for c in x_copies:
        c.start()
    for c in w_copies[1:]:
        c.start()

    w_copies[0].wait()
    for g in range(NG):
        wk_v[:, g * 128:(g + 1) * 128] = wqkv_v[:, D + g * GW:D + g * GW + 128]
    wqvt_v[0:D, :] = wqkv_v[:, 0:D].T
    wqvt_v[D:2 * D, :] = wqkv_v[:, 2 * D:3 * D].T
    qt_v[D:DPAD, :] = jnp.zeros((DPAD - D, S), F32)
    vt_v[D:DPAD, :] = jnp.zeros((DPAD - D, S), F32)

    for r in range(S // RA):
        rows = slice(r * RA, (r + 1) * RA)
        x_copies[r].wait()
        x = x_v[rows, :].astype(F32)
        mu = jnp.mean(x, axis=-1, keepdims=True)
        xc = x - mu
        var = jnp.mean(xc * xc, axis=-1, keepdims=True)
        xn = (xc / jnp.sqrt(var + 1e-5)).astype(BF16)
        xn_v[rows, :] = xn
        kk = _dot(xn, wk_v[...]).astype(BF16)
        for g in range(NG):
            k_v[g, rows, :] = kk[:, g * 128:(g + 1) * 128]
        qv = _dot(wqvt_v[...], xn.T)
        qt_v[0:D, rows] = qv[0:D] * Q_SCALE
        vt_v[0:D, rows] = qv[D:2 * D]

    row32 = lax.broadcasted_iota(jnp.int32, (32, S), 0)
    for h in range(H):
        lo = h * DH - 4 * (h % 2)
        ones_row = DH + 4 * (h % 2)
        va_v[h] = jnp.where(row32 == ones_row, 1.0, vt_v[lo:lo + 32, :]).astype(BF16)

    row128 = lax.broadcasted_iota(jnp.int32, (128, BQ), 0)
    row8 = lax.broadcasted_iota(jnp.int32, (8, BQ), 0)

    def masked_qt(h, qb):
        g = h // HPG
        lo = (h - g * HPG) * DH
        q = qt_v[pl.ds(pl.multiple_of(g * GW, 8), 128), pl.ds(pl.multiple_of(qb * BQ, BQ), BQ)]
        return g, jnp.where((row128 >= lo) & (row128 < lo + DH), q, 0.0).astype(BF16)

    def score_chunk(g, qt, c, dst, m):
        s = _dot(k_v[g, c * CK:(c + 1) * CK, :], qt)
        dst[c * CK:(c + 1) * CK, :] = s
        return jnp.maximum(m, jnp.max(s.reshape(CK // 8, 8, BQ), axis=0))

    def attn_step(h, qb, odd, h_next, qb_next, cur, nxt):
        g, qt = masked_qt(h_next, qb_next)
        m_cur = m_v[...]
        m_next = jnp.full((8, BQ), -jnp.inf, F32)
        acc = jnp.zeros((32, BQ), F32)
        for c in range(S // CK):
            m_next = score_chunk(g, qt, c, nxt, m_next)
            p = jnp.exp2(cur[c * CK:(c + 1) * CK, :] - m_cur).astype(BF16)
            acc = acc + _dot(va_v[h, :, c * CK:(c + 1) * CK], p)
        m_v[...] = jnp.max(m_next, axis=0, keepdims=True)
        cols = pl.ds(pl.multiple_of(qb * BQ, BQ), BQ)
        ones_row = DH + 4 * odd
        o = acc[0:24] / acc[ones_row:ones_row + 1]
        base = pl.multiple_of(h * DH - 4 * odd, 8)
        if odd:
            ot_v[pl.ds(base, 8), cols] = jnp.where(row8 < 4, ot_v[pl.ds(base, 8), cols], o[0:8])
            ot_v[pl.ds(base + 8, 16), cols] = o[8:24]
        else:
            ot_v[pl.ds(base, 24), cols] = o

    g0, qt0 = masked_qt(0, 0)
    m0 = jnp.full((8, BQ), -jnp.inf, F32)
    for c in range(S // CK):
        m0 = score_chunk(g0, qt0, c, sa_v, m0)
    m_v[...] = jnp.max(m0, axis=0, keepdims=True)

    def attn_body(u, carry):
        qb = u // H
        h = u - qb * H
        un = jnp.minimum(u + 1, H * NQB - 1)
        qbn = un // H
        hn = un - qbn * H

        @pl.when(u % 2 == 0)
        def _():
            attn_step(h, qb, 0, hn, qbn, sa_v, sb_v)

        @pl.when(u % 2 == 1)
        def _():
            attn_step(h, qb, 1, hn, qbn, sb_v, sa_v)

        return carry

    lax.fori_loop(0, H * NQB, attn_body, 0)

    for c in w_copies[1:]:
        c.wait()
    out_copies = []
    for r in range(S // RC):
        rows = slice(r * RC, (r + 1) * RC)
        xn = xn_v[rows, :]
        gate = _dot(xn, wg_v[...])
        up = _dot(xn, wu_v[...])
        hid = (gate * jax.nn.sigmoid(gate) * up).astype(BF16)
        o = ot_v[0:D, rows].T.astype(BF16)
        y = x_v[rows, :].astype(F32) + _dot(o, wo_v[...]) + _dot(hid, wd_v[...])
        out_v[rows, :] = y.astype(BF16)
        cp = pltpu.make_async_copy(out_v.at[rows], out_hbm.at[rows], out_sem.at[r])
        cp.start()
        out_copies.append(cp)
    for cp in out_copies:
        cp.wait()


@jax.jit
def pallas_parallel_sum__softmax_full_mha__swiglu_ffn__prompt_kernel(
    A_x: jax.Array,
    A_wqkv: jax.Array,
    A_wo: jax.Array,
    B_x: jax.Array,
    B_w_gate: jax.Array,
    B_w_up: jax.Array,
    B_w_down: jax.Array,
):
    del B_x
    any_spec = pl.BlockSpec(memory_space=pl.ANY)
    out = pl.pallas_call(
        _kernel,
        in_specs=[any_spec] * 6,
        out_specs=any_spec,
        out_shape=jax.ShapeDtypeStruct((S, D), BF16),
        scratch_shapes=[
            pltpu.VMEM((S, D), BF16),
            pltpu.VMEM((D, 3 * D), BF16),
            pltpu.VMEM((D, D), BF16),
            pltpu.VMEM((D, F), BF16),
            pltpu.VMEM((D, F), BF16),
            pltpu.VMEM((F, D), BF16),
            pltpu.VMEM((S, D), BF16),
            pltpu.VMEM((S, D), BF16),
            pltpu.VMEM((D, NG * 128), BF16),
            pltpu.VMEM((2 * D, D), BF16),
            pltpu.VMEM((NG, S, 128), BF16),
            pltpu.VMEM((DPAD, S), F32),
            pltpu.VMEM((DPAD, S), F32),
            pltpu.VMEM((H, 32, S), BF16),
            pltpu.VMEM((DPAD, S), F32),
            pltpu.VMEM((S, BQ), F32),
            pltpu.VMEM((S, BQ), F32),
            pltpu.VMEM((1, BQ), F32),
            pltpu.SemaphoreType.DMA((S // RA + 5,)),
            pltpu.SemaphoreType.DMA((S // RC,)),
        ],
        compiler_params=pltpu.CompilerParams(vmem_limit_bytes=110 * 2**20),
    )(A_x.reshape(S, D), A_wqkv, A_wo, B_w_gate, B_w_up, B_w_down)
    return out.reshape(A_x.shape)
```

```python
import math

import jax
import jax.numpy as jnp
from jax import lax
import jax.experimental.pallas as pl
import jax.experimental.pallas.tpu as pltpu

S, D, F = 2048, 640, 1536
H, DH = 32, 20
HPG = 6
NG = -(-H // HPG)
GW = HPG * DH
DPAD = 768
BQ = 512
NQB = S // BQ
CK = 128
RA = 256
RC = 256
CF = 256
F32, BF16 = jnp.float32, jnp.bfloat16
Q_SCALE = DH ** -0.5 * math.log2(math.e)


def _dot(a, b):
    return lax.dot_general(a, b, (((1,), (0,)), ((), ())), preferred_element_type=F32)


def _kernel(x_hbm, wqkv_hbm, wo_hbm, wg_hbm, wu_hbm, wd_hbm, out_hbm,
            x_v, wqkv_v, wo_v, wg_v, wu_v, wd_v, out_v,
            xn_v, wk_v, wqvt_v, k_v, qt_v, vt_v, ot_v, sa_v, sb_v, m_v, qm_v, hid_v,
            in_sem, out_sem):
    x_copies = [
        pltpu.make_async_copy(x_hbm.at[pl.ds(r * RA, RA)], x_v.at[pl.ds(r * RA, RA)], in_sem.at[r])
        for r in range(S // RA)
    ]
    w_copies = [
        pltpu.make_async_copy(src, dst, in_sem.at[S // RA + i])
        for i, (src, dst) in enumerate(
            [(wqkv_hbm, wqkv_v), (wo_hbm, wo_v), (wg_hbm, wg_v), (wu_hbm, wu_v), (wd_hbm, wd_v)])
    ]
    def layernorm(r):
        rows = pl.ds(pl.multiple_of(r * RA, RA), RA)
        x = x_v[rows, :].astype(F32)
        xc = x - jnp.mean(x, axis=-1, keepdims=True)
        var = jnp.mean(xc * xc, axis=-1, keepdims=True)
        xn_v[rows, :] = (xc * lax.rsqrt(var + 1e-5)).astype(BF16)

    x_copies[0].start()
    w_copies[0].start()
    qt_v[D:DPAD, :] = jnp.zeros((DPAD - D, S), F32)
    x_copies[0].wait()
    x_copies[1].start()
    layernorm(0)

    w_copies[0].wait()
    for c in x_copies[2:] + w_copies[1:]:
        c.start()
    for g in range(NG):
        wk_v[:, g * 128:(g + 1) * 128] = wqkv_v[:, D + g * GW:D + g * GW + 128]
    wqvt_v[0:D, :] = wqkv_v[:, 0:D].T
    wqvt_v[D:2 * D, :] = wqkv_v[:, 2 * D:3 * D].T

    def proj_body(r, carry):
        rows = pl.ds(pl.multiple_of(r * RA, RA), RA)
        nr = jnp.minimum(r + 1, S // RA - 1)
        nrows = pl.ds(pl.multiple_of(nr * RA, RA), RA)

        @pl.when(r + 1 < S // RA)
        def _():
            pltpu.make_async_copy(x_hbm.at[nrows], x_v.at[nrows], in_sem.at[nr]).wait()

        xn = xn_v[rows, :]
        layernorm(nr)
        kk = _dot(xn, wk_v[...]).astype(BF16)
        for g in range(NG):
            k_v[g, rows, :] = kk[:, g * 128:(g + 1) * 128]
        qv = _dot(wqvt_v[...], xn.T)
        qt_v[0:D, rows] = qv[0:D] * Q_SCALE
        vt_v[0:D, rows] = qv[D:2 * D]
        return carry

    lax.fori_loop(0, S // RA, proj_body, 0)

    row128 = lax.broadcasted_iota(jnp.int32, (128, BQ), 0)
    row24 = lax.broadcasted_iota(jnp.int32, (24, CK), 0)
    row8 = lax.broadcasted_iota(jnp.int32, (8, BQ), 0)

    def stage_q(h):
        g = h // HPG
        lo = (h - g * HPG) * DH
        keep = (row128 >= lo) & (row128 < lo + DH)
        for qb in range(NQB):
            cols = slice(qb * BQ, (qb + 1) * BQ)
            q = qt_v[pl.ds(pl.multiple_of(g * GW, 8), 128), cols]
            qm_v[:, cols] = jnp.where(keep, q, 0.0).astype(BF16)

    def attn_step(h, odd, cur, nxt):
        if nxt is not None:
            g = (h + 1) // HPG
        if cur is not None:
            base = pl.multiple_of(h * DH - 4 * odd, 8)
            ones_row = 0 if odd else DH
        for qb in range(NQB):
            cols = slice(qb * BQ, (qb + 1) * BQ)
            if nxt is not None:
                qt = qm_v[:, cols]
                m_next = jnp.full((8, BQ), -jnp.inf, F32)
            if cur is not None:
                m_cur = m_v[:, cols]
                acc = jnp.zeros((24, BQ), F32)
            for c in range(S // CK):
                keys = slice(c * CK, (c + 1) * CK)
                if nxt is not None:
                    s = _dot(k_v[g, keys, :], qt)
                    nxt[keys, cols] = s
                    m_next = jnp.maximum(m_next, jnp.max(s.reshape(CK // 8, 8, BQ), axis=0))
                if cur is not None:
                    p = jnp.exp2(cur[keys, cols] - m_cur).astype(BF16)
                    v = jnp.where(row24 == ones_row, 1.0, vt_v[pl.ds(base, 24), keys])
                    acc = acc + _dot(v, p)
            if nxt is not None:
                m_v[:, cols] = jnp.max(m_next, axis=0, keepdims=True)
            if cur is not None:
                o = acc / acc[ones_row:ones_row + 1]
                if odd:
                    ot_v[pl.ds(base, 8), cols] = jnp.where(
                        row8 < 4, ot_v[pl.ds(base, 8), cols], o[0:8])
                    ot_v[pl.ds(base + 8, 16), cols] = o[8:24]
                else:
                    ot_v[pl.ds(base, 24), cols] = o
        if nxt is not None:
            stage_q(jnp.minimum(h + 2, H - 1))

    stage_q(0)
    attn_step(-1, 1, None, sa_v)

    def attn_body(j, carry):
        attn_step(2 * j, 0, sa_v, sb_v)
        attn_step(2 * j + 1, 1, sb_v, sa_v)
        return carry

    lax.fori_loop(0, H // 2 - 1, attn_body, 0)
    attn_step(H - 2, 0, sa_v, sb_v)
    attn_step(H - 1, 1, sb_v, None)

    for c in w_copies[1:]:
        c.wait()

    def out_copy(r):
        rows = pl.ds(pl.multiple_of(r * RC, RC), RC)
        return pltpu.make_async_copy(out_v.at[rows], out_hbm.at[rows], out_sem.at[r])

    def out_body(r, carry):
        rows = pl.ds(pl.multiple_of(r * RC, RC), RC)
        xn = xn_v[rows, :]
        for c in range(F // CF):
            cols = slice(c * CF, (c + 1) * CF)
            half = 0.5 * _dot(xn, wg_v[:, cols])
            silu = half + half * jnp.tanh(half)
            hid_v[:, cols] = (silu * _dot(xn, wu_v[:, cols])).astype(BF16)
        o = ot_v[0:D, rows].T.astype(BF16)
        y = x_v[rows, :].astype(F32) + _dot(o, wo_v[...]) + _dot(hid_v[...], wd_v[...])
        out_v[rows, :] = y.astype(BF16)
        out_copy(r).start()
        return carry

    lax.fori_loop(0, S // RC, out_body, 0)
    for r in range(S // RC):
        out_copy(r).wait()


@jax.jit
def pallas_parallel_sum__softmax_full_mha__swiglu_ffn__prompt_kernel(
    A_x: jax.Array,
    A_wqkv: jax.Array,
    A_wo: jax.Array,
    B_x: jax.Array,
    B_w_gate: jax.Array,
    B_w_up: jax.Array,
    B_w_down: jax.Array,
):
    del B_x
    any_spec = pl.BlockSpec(memory_space=pl.ANY)
    out = pl.pallas_call(
        _kernel,
        in_specs=[any_spec] * 6,
        out_specs=any_spec,
        out_shape=jax.ShapeDtypeStruct((S, D), BF16),
        scratch_shapes=[
            pltpu.VMEM((S, D), BF16),
            pltpu.VMEM((D, 3 * D), BF16),
            pltpu.VMEM((D, D), BF16),
            pltpu.VMEM((D, F), BF16),
            pltpu.VMEM((D, F), BF16),
            pltpu.VMEM((F, D), BF16),
            pltpu.VMEM((S, D), BF16),
            pltpu.VMEM((S, D), BF16),
            pltpu.VMEM((D, NG * 128), BF16),
            pltpu.VMEM((2 * D, D), BF16),
            pltpu.VMEM((NG, S, 128), BF16),
            pltpu.VMEM((DPAD, S), F32),
            pltpu.VMEM((D, S), F32),
            pltpu.VMEM((D, S), F32),
            pltpu.VMEM((S, S), F32),
            pltpu.VMEM((S, S), F32),
            pltpu.VMEM((1, S), F32),
            pltpu.VMEM((128, S), BF16),
            pltpu.VMEM((RC, F), BF16),
            pltpu.SemaphoreType.DMA((S // RA + 5,)),
            pltpu.SemaphoreType.DMA((S // RC,)),
        ],
        compiler_params=pltpu.CompilerParams(vmem_limit_bytes=110 * 2**20),
    )(A_x.reshape(S, D), A_wqkv, A_wo, B_w_gate, B_w_up, B_w_down)
    return out.reshape(A_x.shape)
```
